```python
import os as _os
_os.environ.setdefault("JAX_PLATFORMS", "cpu")
import jax
import jax.numpy as jnp

def _softmax(x, axis=-1):
    return jax.nn.softmax(x, axis=axis)
def _gelu(x):
    return jax.nn.gelu(x, approximate=True)
def _silu(x):
    return jax.nn.silu(x)
def _sigmoid(x):
    return jax.nn.sigmoid(x)
def _layernorm(x, axis=-1, eps=1e-5):
    m = jnp.mean(x, axis=axis, keepdims=True)
    v = jnp.var(x, axis=axis, keepdims=True)
    return (x - m) / jnp.sqrt(v + eps)
def _scatter_add(tgt, idx, src, axis=0):
    return tgt.at[idx].add(src)
def _segment_sum(src, seg, n):
    return jax.ops.segment_sum(src, seg, n)
class _Rng:
    def __init__(self, key):
        self._k = key
    def _next(self):
        self._k, sub = jax.random.split(self._k)
        return sub
    def normal(self, shape):
        return jax.random.normal(self._next(), shape, dtype=jnp.bfloat16)
    def randint(self, lo, hi, shape):
        return jax.random.randint(self._next(), shape, lo, hi, dtype=jnp.int32)
    def uniform(self, shape, lo=0.0, hi=1.0):
        return jax.random.uniform(self._next(), shape, jnp.bfloat16, lo, hi)
    def permutation(self, n):
        return jax.random.permutation(self._next(), n)


kernel_name = 'interleave_layers__linear_kernel_hedgehog__dense_activation_silu__prompt'

def setup_inputs():
    _rng = _Rng(jax.random.key(int.from_bytes(__import__("os").urandom(4), "little")))
    _w = (lambda a: (lambda t: t.astype(jnp.bfloat16) if jnp.issubdtype(t.dtype, jnp.floating) else t)(jnp.asarray(a)))
    def _A_setup():
        B, S, D, H = 1, 2048, 640, 32
        Dh = D // H
        return {
            "x": _w((lambda *s: _rng.normal(s) * 0.05)(B, S, D)),
            "wqkv": _w((lambda *s: _rng.normal(s) * 0.4)(D, 3 * D)),
            "w_phi": _w((lambda *s: _rng.normal(s) * 0.4)(H, Dh, Dh) * (Dh ** -0.5)),
            "wo": _w((lambda *s: _rng.normal(s) * 0.05)(D, D)),
        }
    _A_in = _A_setup()

    def _B_setup():
        B, S, D, F = 1, 2048, 640, 1728
        return {
            "x": _w((lambda *s: _rng.normal(s) * 0.05)(B, S, D)),
            "w1": _w((lambda *s: _rng.normal(s) * 1.6)(D, F) * (D ** -0.5)),
            "w2": _w((lambda *s: _rng.normal(s) * 1.6)(F, D) * (F ** -0.5)),
        }
    _B_in = _B_setup()

    return {
        "A_x": _A_in["x"],
        "A_wqkv": _A_in["wqkv"],
        "A_w_phi": _A_in["w_phi"],
        "A_wo": _A_in["wo"],
        "B_x": _B_in["x"],
        "B_w1": _B_in["w1"],
        "B_w2": _B_in["w2"],
    }

def reference(A_x, A_wqkv, A_w_phi, A_wo, B_x, B_w1, B_w2):
    def _A_ref(x, wqkv, w_phi, wo):
        B, S, D = x.shape
        H = 32; Dh = D // H
        qkv = (lambda x, *d: x.transpose(*d))((x @ wqkv).reshape(B, S, 3, H, Dh), 2, 0, 3, 1, 4)
        q, k, v = qkv[0], qkv[1], qkv[2]
        pq = jnp.einsum("bhsd,hdf->bhsf", q, w_phi)
        pk = jnp.einsum("bhsd,hdf->bhsf", k, w_phi)
        phi_q = jnp.concatenate([_softmax(pq, axis=-1), _softmax(-pq, axis=-1)], axis=-1)
        phi_k = jnp.concatenate([_softmax(pk, axis=-1), _softmax(-pk, axis=-1)], axis=-1)
        kv = jnp.einsum("bhsf,bhsd->bhfd", phi_k, v)
        z  = jnp.einsum("bhsf->bhf", phi_k)
        num = jnp.einsum("bhqf,bhfd->bhqd", phi_q, kv)
        den = jnp.einsum("bhqf,bhf->bhq", phi_q, z)[..., None] + 1e-6
        o = num / den
        return (lambda x, *d: x.transpose(*d))(o, 0, 2, 1, 3).reshape(B, S, D) @ wo

    def _B_ref(x, w1, w2):
        h = jnp.einsum("bsd,df->bsf", x, w1)
        h = _silu(h)
        out = jnp.einsum("bsf,fd->bsd", h, w2)
        return out

    x = A_x
    x = x + _A_ref(_layernorm(x, axis=-1), A_wqkv, A_w_phi, A_wo)
    x = x + _B_ref(_layernorm(x, axis=-1), B_w1, B_w2)
    x = x + _A_ref(_layernorm(x, axis=-1), A_wqkv, A_w_phi, A_wo)
    x = x + _B_ref(_layernorm(x, axis=-1), B_w1, B_w2)
    return x
```

```python
import jax
import jax.numpy as jnp
from jax import lax
import jax.experimental.pallas as pl
import jax.experimental.pallas.tpu as pltpu

F32 = jnp.float32
BF16 = jnp.bfloat16
H = 32
HG = 2
NG = H // HG
T1, T2, T3 = 512, 512, 512

NT = (((1,), (1,)), ((), ()))


def _dot(a, b):
    return jnp.dot(a, b, preferred_element_type=F32)


def _dot_nt(a, b):
    return lax.dot_general(a, b, NT, preferred_element_type=F32)


def _iota(shape, d):
    return lax.broadcasted_iota(jnp.int32, shape, d)


def _ln(x, axis=0):
    m = jnp.mean(x, axis=axis, keepdims=True)
    c = x - m
    v = jnp.mean(c * c, axis=axis, keepdims=True)
    return (c * lax.rsqrt(v + 1e-5)).astype(BF16)


def _fold(op, r):
    sh = 4
    while sh >= HG:
        r = op(r, pltpu.roll(r, sh, r.ndim - 2))
        sh //= 2
    return r


def _phi(p):
    d, t = p.shape
    p = p.reshape(NG, d // NG // 8, 8, t)
    mx = _fold(jnp.maximum, jnp.max(p, axis=1, keepdims=True))
    mn = _fold(jnp.minimum, jnp.min(p, axis=1, keepdims=True))
    ep = jnp.exp2(p - mx)
    en = jnp.exp2(mn - p)
    ep = ep * (1.0 / _fold(jnp.add, jnp.sum(ep, axis=1, keepdims=True)))
    en = en * (1.0 / _fold(jnp.add, jnp.sum(en, axis=1, keepdims=True)))
    return jnp.concatenate([ep, en], axis=1).reshape(NG, 2 * d // NG, t).astype(BF16)


def _kernel(x_hbm, wqkv_hbm, wphi_hbm, wo_hbm, w1_hbm, w2_hbm, out_hbm,
            xin, xres, wqkv, wphi, wo, w1, w2, wt, wot, w2t, phiq, kvacc, kvm, obuf, sems, osem, xsem):
    D, S = xres.shape
    dh = D // H
    gw = dh * HG
    ge = gw + 8
    nt = S // T1

    def mk(sem, s, d):
        return pltpu.make_async_copy(s, d, sem)
    c_phi = mk(sems.at[0], wphi_hbm, wphi)

    def c_qkv(j):
        cs = pl.ds(pl.multiple_of(j * D, 128), D)
        return mk(sems.at[1 + j], wqkv_hbm.at[:, cs], wqkv.at[:, cs])
    c_wo = mk(sems.at[4], wo_hbm, wo)
    c_w1 = mk(sems.at[5], w1_hbm, w1)
    c_w2 = mk(sems.at[6], w2_hbm, w2)
    nc = D // 128

    def c_x(i):
        ts = pl.ds(pl.multiple_of(i * T1, T1), T1)
        return mk(xsem.at[i], x_hbm.at[ts, :], xin.at[ts, :])

    c_phi.start()
    for j in range(3):
        c_qkv(j).start()
    c_x(0).start()
    c_phi.wait()
    assert D == 640 and gw == 40
    pg = 4 * gw
    LOG2E = 1.4426950408889634
    wp = wphi[...].astype(F32).transpose(1, 2, 0).reshape(dh, D)
    row = _iota((pg, 128), 0)
    col = _iota((pg, 128), 1)
    bds = []
    for t in range(nc):
        b = jnp.broadcast_to(wp[None, :, None, t * 128:(t + 1) * 128], (4, dh, HG, 128)).reshape(pg, 128)
        hm = ((col + t * 128) // dh) == ((3 * t + row // gw) * HG + row % HG)
        bds.append(jnp.where(hm, b, 0.0).astype(BF16))

    @pl.loop(0, 2)
    def _(j):
        c_qkv(j).wait()
        parts = []
        for t in range(nc):
            rt = _dot_nt(bds[t], wqkv[:, pl.ds(pl.multiple_of(j * D + t * 128, 128), 128)]) * LOG2E
            if t > 0:
                parts.append(prev + rt[:gw])
            else:
                parts.append(rt[:gw])
            parts.append(rt[gw:3 * gw])
            prev = rt[3 * gw:]
        parts.append(prev)
        wt[pl.ds(pl.multiple_of(j * D, 128), D), :] = jnp.concatenate(parts, axis=0).astype(BF16)
    c_qkv(2).wait()
    for i in range(1, nt):
        c_x(i).start()
    wt[2 * D:3 * D, :] = wqkv[:, 2 * D:3 * D].T

    c_w2.start()
    c_wo.start()
    c_w1.start()
    kvacc[...] = jnp.zeros_like(kvacc)

    def attn_in(i, xn, T, dot):
        ts = pl.ds(pl.multiple_of(i * T, T), T)
        ones = jnp.ones((8, T), F32)
        vt = dot(wt[2 * D:3 * D, :], xn)
        ph = _phi(dot(wt[D:2 * D, :], xn))
        phiq[:, :, ts] = _phi(dot(wt[0:D, :], xn))
        for g in range(NG):
            ve = jnp.concatenate([vt[g * gw:(g + 1) * gw], ones], axis=0).astype(BF16)
            kvacc[g] += _dot_nt(ve, ph[g])

    def finish_kv():
        r = _iota((ge, 2 * gw), 0)
        c = _iota((ge, 2 * gw), 1)
        m = jnp.where(r < gw, r // dh, r % HG) == (c % HG)
        for g in range(NG):
            kvm[g] = jnp.where(m, kvacc[g], 0.0).astype(BF16)

    def attn_out_ffn(i, T, first):
        ts = pl.ds(pl.multiple_of(i * T, T), T)
        os_ = []
        for g in range(NG):
            nd = _dot(kvm[g], phiq[g, :, ts])
            den = nd[gw:gw + 8] + 1e-6
            rd = 1.0 / den
            rs = pltpu.roll(rd, 1, 0)
            ev = _iota((8, T), 0) % 2 == 0
            r0 = jnp.where(ev, rd, rs)
            r1 = jnp.where(ev, rs, rd)
            rm = jnp.where(_iota((8, T), 0) < 4, r0, r1)
            os_.append(nd[:gw] * jnp.concatenate([r0, r0, rm, r1, r1], axis=0))
        o = jnp.concatenate(os_, axis=0).astype(BF16)
        res = xin[ts, :].astype(F32).T if first else xres[:, ts]
        x = res + _dot(wot[...], o)
        h = _dot(w1[...], _ln(x))
        h = (h * jax.nn.sigmoid(h)).astype(BF16)
        return x + _dot(w2t[...], h)

    @pl.loop(0, S // T1)
    def _(i):
        ts = pl.ds(pl.multiple_of(i * T1, T1), T1)
        c_x(i).wait()
        attn_in(i, _ln(xin[ts, :].astype(F32), axis=1), T1, _dot_nt)

    c_w1.wait()
    c_wo.wait()
    c_w2.wait()
    eye = jnp.where(_iota((128, 128), 0) == _iota((128, 128), 1), 1.0, 0.0).astype(BF16)
    for t in range(nc):
        cs = slice(t * 128, (t + 1) * 128)
        if t < 3:
            w2t[cs, :] = _dot_nt(eye, w2[:, cs]).astype(BF16)
        else:
            w2t[cs, :] = w2[:, cs].T
    wot[...] = wo[...].T
    finish_kv()
    kvacc[...] = jnp.zeros_like(kvacc)

    @pl.loop(0, S // T2)
    def _(i):
        ts = pl.ds(pl.multiple_of(i * T2, T2), T2)
        x = attn_out_ffn(i, T2, True)
        xres[:, ts] = x
        attn_in(i, _ln(x), T2, _dot)

    finish_kv()

    @pl.loop(0, S // T3)
    def _(i):
        y = attn_out_ffn(i, T3, False)
        C = T3 // 4
        for c in range(T3 // C):
            ts = pl.ds(pl.multiple_of(i * T3 + c * C, C), C)
            obuf[ts, :] = y[:, c * C:(c + 1) * C].T.astype(obuf.dtype)
            pltpu.make_async_copy(obuf.at[ts, :], out_hbm.at[ts, :], osem).start()

    pltpu.make_async_copy(obuf, out_hbm, osem).wait()


@jax.jit
def pallas_interleave_layers__linear_kernel_hedgehog__dense_activation_silu__prompt_kernel(
    A_x, A_wqkv, A_w_phi, A_wo, B_x, B_w1, B_w2,
):
    B, S, D = A_x.shape
    assert B == 1
    dh = D // H
    gw = dh * HG
    x = A_x.reshape(S, D)
    wphi = A_w_phi.transpose(1, 2, 0)
    dt = A_x.dtype
    any_spec = pl.BlockSpec(memory_space=pltpu.HBM)
    out = pl.pallas_call(
        _kernel,
        out_shape=jax.ShapeDtypeStruct((S, D), dt),
        in_specs=[any_spec] * 6,
        out_specs=any_spec,
        scratch_shapes=[
            pltpu.VMEM((S, D), dt),
            pltpu.VMEM((D, S), F32),
            pltpu.VMEM(A_wqkv.shape, BF16),
            pltpu.VMEM(wphi.shape, BF16),
            pltpu.VMEM(A_wo.shape, BF16),
            pltpu.VMEM(B_w1.shape[::-1], BF16),
            pltpu.VMEM(B_w2.shape, BF16),
            pltpu.VMEM((3 * D, D), BF16),
            pltpu.VMEM((D, D), BF16),
            pltpu.VMEM(B_w2.shape[::-1], BF16),
            pltpu.VMEM((NG, 2 * gw, S), BF16),
            pltpu.VMEM((NG, gw + 8, 2 * gw), F32),
            pltpu.VMEM((NG, gw + 8, 2 * gw), BF16),
            pltpu.VMEM((S, D), dt),
            pltpu.SemaphoreType.DMA((7,)),
            pltpu.SemaphoreType.DMA,
            pltpu.SemaphoreType.DMA((S // T1,)),
        ],
        compiler_params=pltpu.CompilerParams(vmem_limit_bytes=100 * 1024 * 1024),
    )(x, A_wqkv, wphi, A_wo, B_w1.T, B_w2)
    return out.reshape(B, S, D)
```
